```python
import jax
import jax.numpy as jnp

def _softmax(x, axis=-1):
    return jax.nn.softmax(x, axis=axis)

def _gelu(x):
    return jax.nn.gelu(x, approximate=True)

def _silu(x):
    return jax.nn.silu(x)

def _sigmoid(x):
    return jax.nn.sigmoid(x)

def _layernorm(x, axis=-1, eps=1e-05):
    m = jnp.mean(x, axis=axis, keepdims=True)
    v = jnp.var(x, axis=axis, keepdims=True)
    return (x - m) / jnp.sqrt(v + eps)

def _scatter_add(tgt, idx, src, axis=0):
    return tgt.at[idx].add(src)

def _segment_sum(src, seg, n):
    return jax.ops.segment_sum(src, seg, n)

class _Rng:

    def __init__(self, key):
        self._k = key

    def _next(self):
        self._k, sub = jax.random.split(self._k)
        return sub

    def normal(self, shape):
        return jax.random.normal(self._next(), shape, dtype=jnp.bfloat16)

    def randint(self, lo, hi, shape):
        return jax.random.randint(self._next(), shape, lo, hi, dtype=jnp.int32)

    def uniform(self, shape, lo=0.0, hi=1.0):
        return jax.random.uniform(self._next(), shape, jnp.bfloat16, lo, hi)

    def permutation(self, n):
        return jax.random.permutation(self._next(), n)
kernel_name = 'adaLN_cond__sliding_block_cached__glu_gated_bilinear__decode'

def setup_inputs():
    _rng = _Rng(jax.random.key(int.from_bytes(__import__("os").urandom(4), "little")))
    _w = lambda a: (lambda t: t.astype(jnp.bfloat16) if jnp.issubdtype(t.dtype, jnp.floating) else t)(jnp.asarray(a))

    def _A_setup():
        B, Sq, D = (1, 1, 640)
        Hq, Hkv, Sk, Dh = (32, 32, 32768, 192)
        assert Hq % Hkv == 0, (Hq, Hkv)
        return {'x': _w((lambda *s: _rng.normal(s) * 0.05)(B, Sq, D)), 'k_cache': _w((lambda *s: _rng.normal(s) * 0.05)(B, Hkv, Sk, Dh)), 'v_cache': _w((lambda *s: _rng.normal(s) * 0.05)(B, Hkv, Sk, Dh)), 'wq': _w((lambda *s: _rng.normal(s) * 0.05)(D, Hq * Dh) * D ** (-0.5)), 'wo': _w((lambda *s: _rng.normal(s) * 0.05)(Hq * Dh, D) * (Hq * Dh) ** (-0.5))}
    _A_in = _A_setup()

    def _B_setup():
        B, S, D, F = (1, 1, 640, 1536)
        return {'x': _w((lambda *s: _rng.normal(s) * 0.05)(B, S, D)), 'w_gate': _w((lambda *s: _rng.normal(s) * 0.05)(D, F) * D ** (-0.5)), 'w_up': _w((lambda *s: _rng.normal(s) * 0.05)(D, F) * D ** (-0.5)), 'w_down': _w((lambda *s: _rng.normal(s) * 0.05)(F, D) * F ** (-0.5))}
    _B_in = _B_setup()
    return {'A_x': _A_in['x'], 'A_k_cache': _A_in['k_cache'], 'A_v_cache': _A_in['v_cache'], 'A_wq': _A_in['wq'], 'A_wo': _A_in['wo'], 'B_x': _B_in['x'], 'B_w_gate': _B_in['w_gate'], 'B_w_up': _B_in['w_up'], 'B_w_down': _B_in['w_down'], 'c': _w((lambda *s: _rng.normal(s) * 0.05)(1, 640)), 'w_mod': _w((lambda *s: _rng.normal(s) * 0.05)(640, 6 * 640) * 640 ** (-0.5))}

def reference(A_x, A_k_cache, A_v_cache, A_wq, A_wo, B_x, B_w_gate, B_w_up, B_w_down, c, w_mod):

    def _A_ref(x, k_cache, v_cache, wq, wo):
        B, Sq, D = x.shape
        Hq, Dh = (32, 192)
        Hkv, Sk = (k_cache.shape[1], k_cache.shape[2])
        W = min(4096, max(256, Sk // 4))
        rep = Hq // Hkv
        q = (lambda x, *d: x.transpose(*d))((x @ wq).reshape(B, Sq, Hq, Dh), 0, 2, 1, 3)
        k = jnp.repeat(k_cache[:, :, Sk - W:, :], rep, axis=1)
        v = jnp.repeat(v_cache[:, :, Sk - W:, :], rep, axis=1)
        scores = jnp.einsum('bhqd,bhkd->bhqk', q, k) * Dh ** (-0.5)
        p = _softmax(scores, axis=-1)
        o = jnp.einsum('bhqk,bhkd->bhqd', p, v)
        return (lambda x, *d: x.transpose(*d))(o, 0, 2, 1, 3).reshape(B, Sq, Hq * Dh) @ wo

    def _B_ref(x, w_gate, w_up, w_down):
        g = jnp.einsum('bsd,df->bsf', x, w_gate)
        u = jnp.einsum('bsd,df->bsf', x, w_up)
        h = g * u
        return jnp.einsum('bsf,fd->bsd', h, w_down)
    x = A_x
    mod = (_silu(c) @ w_mod).reshape(c.shape[0], 6, 1, -1)
    sa, ca, ga, sb, cb, gb = (mod[:, 0].copy(), mod[:, 1].copy(), mod[:, 2].copy(), mod[:, 3].copy(), mod[:, 4].copy(), mod[:, 5].copy())
    h = _layernorm(x, axis=-1) * (1 + ca) + sa
    x = x + ga * _A_ref(h, A_k_cache, A_v_cache, A_wq, A_wo)
    h = _layernorm(x, axis=-1) * (1 + cb) + sb
    x = x + gb * _B_ref(h, B_w_gate, B_w_up, B_w_down)
    return x
```

```python
import functools

import jax
import jax.numpy as jnp
from jax import lax
from jax.experimental import pallas as pl
from jax.experimental.pallas import tpu as pltpu

_HQ, _DH = 32, 192
_G = 8
_NS = 2


def _dot(a, b):
    return jnp.dot(a, b, preferred_element_type=jnp.float32)


def _dot_nt(a, b):
    return lax.dot_general(a, b, (((1,), (1,)), ((), ())), preferred_element_type=jnp.float32)


def _ln(x):
    m = jnp.mean(x, axis=-1, keepdims=True)
    d = x - m
    v = jnp.mean(d * d, axis=-1, keepdims=True)
    return d * lax.rsqrt(v + 1e-5)


def _kernel(x_hbm, kT, vT, wq_hbm, wo_hbm, wg_hbm, wu_hbm, wd_hbm, c_hbm, wm_hbm, o_ref,
            x_v, c_v, wm_v, wq_v, wg_v, wu_v, wd_v, kbuf, vbuf, wobuf, q_scr, sw, sk, sv, so, *, S0, W):
    G, NS = _G, _NS
    NG = _HQ // G
    GD = G * _DH
    D = x_v.shape[-1]

    def kcp(g, slot):
        return pltpu.make_async_copy(kT.at[pl.ds(pl.multiple_of(g * GD, 16), GD), pl.ds(S0, W)], kbuf.at[slot], sk.at[slot])

    def vcp(g, slot):
        return pltpu.make_async_copy(vT.at[pl.ds(pl.multiple_of(g * GD, 16), GD), pl.ds(S0, W)], vbuf.at[slot], sv.at[slot])

    def ocp(g, slot):
        return pltpu.make_async_copy(wo_hbm.at[pl.ds(pl.multiple_of(g * GD, 16), GD), :], wobuf.at[slot], so.at[slot])

    cp_c = pltpu.make_async_copy(c_hbm, c_v, sw.at[0])
    cp_x = pltpu.make_async_copy(x_hbm, x_v, sw.at[1])
    cp_wm = pltpu.make_async_copy(wm_hbm, wm_v, sw.at[2])
    cp_wq = pltpu.make_async_copy(wq_hbm, wq_v, sw.at[3])
    cp_wg = pltpu.make_async_copy(wg_hbm, wg_v, sw.at[4])
    cp_wu = pltpu.make_async_copy(wu_hbm, wu_v, sw.at[5])
    cp_wd = pltpu.make_async_copy(wd_hbm, wd_v, sw.at[6])

    cp_c.start(); cp_x.start(); cp_wm.start(); cp_wq.start()
    for g in range(NS):
        kcp(g, g).start(); vcp(g, g).start(); ocp(g, g).start()

    cp_c.wait(); cp_wm.wait()
    cc = c_v[...].astype(jnp.float32)
    sc = (cc * jax.nn.sigmoid(cc)).astype(jnp.bfloat16)
    mod = _dot(sc, wm_v[...])
    sa, ca, ga = mod[:, 0:D], mod[:, D:2 * D], mod[:, 2 * D:3 * D]
    sb, cb, gb = mod[:, 3 * D:4 * D], mod[:, 4 * D:5 * D], mod[:, 5 * D:6 * D]
    cp_x.wait()
    x = x_v[...].astype(jnp.float32)
    h = (_ln(x) * (1.0 + ca) + sa).astype(jnp.bfloat16)
    h8 = jnp.broadcast_to(h, (8, D))
    row = lax.broadcasted_iota(jnp.int32, (8, GD), 0)
    col = lax.broadcasted_iota(jnp.int32, (8, GD), 1)
    bd = (col >= row * _DH) & (col < (row + 1) * _DH)
    cp_wq.wait()
    for g in range(NG):
        qg = _dot(h8, wq_v[:, g * GD:(g + 1) * GD])
        q_scr[g] = jnp.where(bd, qg, 0.0).astype(jnp.bfloat16)

    scale = _DH ** -0.5

    def body(g, acc):
        slot = g % NS
        kcp(g, slot).wait()
        s = _dot(q_scr[g], kbuf[slot]) * scale

        @pl.when(g + NS < NG)
        def _():
            kcp(g + NS, slot).start()

        @pl.when(g + NS == NG)
        def _():
            cp_wg.start()
        m = jnp.max(s, axis=-1, keepdims=True)
        p = jnp.exp(s - m)
        l = jnp.sum(p, axis=-1, keepdims=True)
        vcp(g, slot).wait()
        o = _dot_nt(p.astype(jnp.bfloat16), vbuf[slot])

        @pl.when(g + NS < NG)
        def _():
            vcp(g + NS, slot).start()

        @pl.when(g + NS == NG)
        def _():
            cp_wu.start()
        o = jnp.where(bd, o * (1.0 / l), 0.0).astype(jnp.bfloat16)
        ocp(g, slot).wait()
        acc = acc + _dot(o, wobuf[slot])

        @pl.when(g + NS < NG)
        def _():
            ocp(g + NS, slot).start()

        @pl.when(g + NS == NG)
        def _():
            cp_wd.start()
        return acc

    acc = lax.fori_loop(0, NG, body, jnp.zeros((8, D), jnp.float32))
    attn = jnp.sum(acc, axis=0, keepdims=True)
    x1 = x + ga * attn
    h2 = (_ln(x1) * (1.0 + cb) + sb).astype(jnp.bfloat16)
    cp_wg.wait()
    gg = _dot(h2, wg_v[...])
    cp_wu.wait()
    uu = _dot(h2, wu_v[...])
    hh = (gg * uu).astype(jnp.bfloat16)
    cp_wd.wait()
    y = _dot(hh, wd_v[...])
    o_ref[...] = (x1 + gb * y).astype(o_ref.dtype)


@jax.jit
def pallas_adaLN_cond__sliding_block_cached__glu_gated_bilinear__decode_kernel(
    A_x: jax.Array,
    A_k_cache: jax.Array,
    A_v_cache: jax.Array,
    A_wq: jax.Array,
    A_wo: jax.Array,
    B_x: jax.Array,
    B_w_gate: jax.Array,
    B_w_up: jax.Array,
    B_w_down: jax.Array,
    c: jax.Array,
    w_mod: jax.Array,
):
    del B_x
    B, Sq, D = A_x.shape
    _, Hkv, Sk, Dh = A_k_cache.shape
    assert (B, Sq) == (1, 1) and (Hkv, Dh) == (_HQ, _DH)
    W = min(4096, max(256, Sk // 4))
    F = B_w_gate.shape[1]
    GD = _G * _DH
    kT = jnp.swapaxes(A_k_cache.reshape(Hkv, Sk, Dh), 1, 2).reshape(Hkv * Dh, Sk)
    vT = jnp.swapaxes(A_v_cache.reshape(Hkv, Sk, Dh), 1, 2).reshape(Hkv * Dh, Sk)
    x2 = A_x.reshape(1, D)
    bf = jnp.bfloat16
    out = pl.pallas_call(
        functools.partial(_kernel, S0=Sk - W, W=W),
        out_shape=jax.ShapeDtypeStruct((1, D), A_x.dtype),
        in_specs=[pl.BlockSpec(memory_space=pl.ANY)] * 10,
        out_specs=pl.BlockSpec(memory_space=pltpu.VMEM),
        scratch_shapes=[
            pltpu.VMEM((1, D), bf), pltpu.VMEM((1, D), bf),
            pltpu.VMEM((D, 6 * D), bf), pltpu.VMEM((D, _HQ * _DH), bf),
            pltpu.VMEM((D, F), bf), pltpu.VMEM((D, F), bf), pltpu.VMEM((F, D), bf),
            pltpu.VMEM((_NS, GD, W), bf), pltpu.VMEM((_NS, GD, W), bf), pltpu.VMEM((_NS, GD, D), bf),
            pltpu.VMEM((_HQ // _G, 8, GD), bf),
            pltpu.SemaphoreType.DMA((7,)), pltpu.SemaphoreType.DMA((_NS,)),
            pltpu.SemaphoreType.DMA((_NS,)), pltpu.SemaphoreType.DMA((_NS,)),
        ],
        compiler_params=pltpu.CompilerParams(vmem_limit_bytes=100 * 1024 * 1024),
    )(x2, kT, vT, A_wq, A_wo, B_w_gate, B_w_up, B_w_down, c, w_mod)
    return out.reshape(B, Sq, D)
```

```python
import functools

import jax
import jax.numpy as jnp
from jax import lax
from jax.experimental import pallas as pl
from jax.experimental.pallas import tpu as pltpu

_HQ, _DH = 32, 192
_G = 4
_NS = 2
_M = 8
_WD_ROWS = 128
_EPS = 1e-5


def _dot(a, b):
    return jnp.dot(a, b, preferred_element_type=jnp.float32)


def _dot_nt(a, b):
    return lax.dot_general(a, b, (((1,), (1,)), ((), ())), preferred_element_type=jnp.float32)


def _layernorm(x):
    d = x - jnp.mean(x, axis=-1, keepdims=True)
    v = jnp.mean(d * d, axis=-1, keepdims=True)
    return d * lax.rsqrt(v + _EPS)


def _kernel(x_hbm, kT_hbm, vT_hbm, wq_hbm, wo_hbm, wg_hbm, wu_hbm, wd_hbm, c_hbm, wm_hbm,
            o_ref,
            x_v, c_v, wm_v, wq_v, wg_v, wu_v, wd_v, k_buf, v_buf, wo_buf, q_scr, hh_scr,
            sem_w, sem_k, sem_v, sem_o, sem_d, *, s0, w):
    f32, bf16 = jnp.float32, jnp.bfloat16
    n_groups = _HQ // _G
    gd = _G * _DH
    d = x_v.shape[-1]
    n_wd = wd_v.shape[0] // _WD_ROWS

    def group_rows(g):
        return pl.ds(pl.multiple_of(g * gd, 16), gd)

    def k_copy(g, slot):
        return pltpu.make_async_copy(kT_hbm.at[group_rows(g), pl.ds(s0, w)], k_buf.at[slot], sem_k.at[slot])

    def v_copy(g, slot):
        return pltpu.make_async_copy(vT_hbm.at[group_rows(g), pl.ds(s0, w)], v_buf.at[slot], sem_v.at[slot])

    def wo_copy(g, slot):
        return pltpu.make_async_copy(wo_hbm.at[group_rows(g), :], wo_buf.at[slot], sem_o.at[slot])

    def wd_copy(i):
        rows = pl.ds(pl.multiple_of(i * _WD_ROWS, _WD_ROWS), _WD_ROWS)
        return pltpu.make_async_copy(wd_hbm.at[rows, :], wd_v.at[rows, :], sem_d.at[i])

    wm_copy = pltpu.make_async_copy(wm_hbm, wm_v, sem_w.at[0])
    c_copy = pltpu.make_async_copy(c_hbm, c_v, sem_w.at[1])
    x_copy = pltpu.make_async_copy(x_hbm, x_v, sem_w.at[2])
    wq_copy = pltpu.make_async_copy(wq_hbm, wq_v, sem_w.at[3])
    wg_copy = pltpu.make_async_copy(wg_hbm, wg_v, sem_w.at[4])
    wu_copy = pltpu.make_async_copy(wu_hbm, wu_v, sem_w.at[5])

    wm_copy.start()
    c_copy.start()
    x_copy.start()
    wq_copy.start()
    for g in range(_NS):
        k_copy(g, g).start()
        v_copy(g, g).start()
        wo_copy(g, g).start()

    c_copy.wait()
    wm_copy.wait()
    cc = jnp.broadcast_to(c_v[...].astype(f32), (_M, d))
    mod = _dot((cc * jax.nn.sigmoid(cc)).astype(bf16), wm_v[...])
    sa, ca, ga, sb, cb, gb = (mod[:, i * d:(i + 1) * d] for i in range(6))

    x_copy.wait()
    x = jnp.broadcast_to(x_v[...].astype(f32), (_M, d))
    h = (_layernorm(x) * (1.0 + ca) + sa).astype(bf16)

    row = lax.broadcasted_iota(jnp.int32, (_M, gd), 0)
    col = lax.broadcasted_iota(jnp.int32, (_M, gd), 1)
    block_diag = (col >= row * _DH) & (col < (row + 1) * _DH)
    wq_copy.wait()
    for g in range(n_groups):
        q = _dot(h, wq_v[:, g * gd:(g + 1) * gd])
        q_scr[g] = jnp.where(block_diag, q, 0.0).astype(bf16)

    def attend(g, acc):
        slot = g % _NS
        refill = g + _NS < n_groups

        k_copy(g, slot).wait()
        s = _dot(q_scr[g], k_buf[slot]) * (_DH ** -0.5)

        @pl.when(refill)
        def _():
            k_copy(g + _NS, slot).start()

        @pl.when(g + _NS == n_groups)
        def _():
            wg_copy.start()
            wu_copy.start()

            @pl.loop(0, n_wd)
            def _(i):
                wd_copy(i).start()

        p = jnp.exp(s - jnp.max(s, axis=-1, keepdims=True))
        denom = jnp.sum(p, axis=-1, keepdims=True)

        v_copy(g, slot).wait()
        o = _dot_nt(p.astype(bf16), v_buf[slot])

        @pl.when(refill)
        def _():
            v_copy(g + _NS, slot).start()

        o = jnp.where(block_diag, o * (1.0 / denom), 0.0).astype(bf16)

        wo_copy(g, slot).wait()
        acc = acc + _dot(o, wo_buf[slot])

        @pl.when(refill)
        def _():
            wo_copy(g + _NS, slot).start()

        return acc

    acc = lax.fori_loop(0, n_groups, attend, jnp.zeros((_M, d), f32))
    attn = jnp.broadcast_to(jnp.sum(acc, axis=0, keepdims=True), (_M, d))
    x1 = x + ga * attn

    h2 = (_layernorm(x1) * (1.0 + cb) + sb).astype(bf16)
    wg_copy.wait()
    gate = _dot(h2, wg_v[...])
    wu_copy.wait()
    up = _dot(h2, wu_v[...])
    hh = (gate * up).astype(bf16)
    for i in range(n_wd):
        hh_scr[i] = hh[:, i * _WD_ROWS:(i + 1) * _WD_ROWS]

    def down(i, y):
        wd_copy(i).wait()
        rows = pl.ds(pl.multiple_of(i * _WD_ROWS, _WD_ROWS), _WD_ROWS)
        return y + _dot(hh_scr[i], wd_v[rows, :])

    y = lax.fori_loop(0, n_wd, down, jnp.zeros((_M, d), f32))
    o_ref[...] = (x1 + gb * y)[0:1, :].astype(o_ref.dtype)


@jax.jit
def pallas_adaLN_cond__sliding_block_cached__glu_gated_bilinear__decode_kernel(
    A_x: jax.Array,
    A_k_cache: jax.Array,
    A_v_cache: jax.Array,
    A_wq: jax.Array,
    A_wo: jax.Array,
    B_x: jax.Array,
    B_w_gate: jax.Array,
    B_w_up: jax.Array,
    B_w_down: jax.Array,
    c: jax.Array,
    w_mod: jax.Array,
):
    del B_x
    batch, sq, d = A_x.shape
    _, hkv, sk, dh = A_k_cache.shape
    f = B_w_gate.shape[1]
    w = min(4096, max(256, sk // 4))
    gd = _G * _DH
    assert (batch, sq) == (1, 1) and (hkv, dh) == (_HQ, _DH)
    assert gd % 128 == 0 and _G <= _M and _HQ % _G == 0 and f % _WD_ROWS == 0
    assert w % 128 == 0 and (sk - w) % 128 == 0

    kT = jnp.swapaxes(A_k_cache.reshape(hkv, sk, dh), 1, 2).reshape(hkv * dh, sk)
    vT = jnp.swapaxes(A_v_cache.reshape(hkv, sk, dh), 1, 2).reshape(hkv * dh, sk)

    bf16 = jnp.bfloat16
    dma = pltpu.SemaphoreType.DMA
    out = pl.pallas_call(
        functools.partial(_kernel, s0=sk - w, w=w),
        out_shape=jax.ShapeDtypeStruct((1, d), A_x.dtype),
        in_specs=[pl.BlockSpec(memory_space=pl.ANY)] * 10,
        out_specs=pl.BlockSpec(memory_space=pltpu.VMEM),
        scratch_shapes=[
            pltpu.VMEM((1, d), bf16),
            pltpu.VMEM((1, d), bf16),
            pltpu.VMEM((d, 6 * d), bf16),
            pltpu.VMEM((d, _HQ * _DH), bf16),
            pltpu.VMEM((d, f), bf16),
            pltpu.VMEM((d, f), bf16),
            pltpu.VMEM((f, d), bf16),
            pltpu.VMEM((_NS, gd, w), bf16),
            pltpu.VMEM((_NS, gd, w), bf16),
            pltpu.VMEM((_NS, gd, d), bf16),
            pltpu.VMEM((_HQ // _G, _M, gd), bf16),
            pltpu.VMEM((f // _WD_ROWS, _M, _WD_ROWS), bf16),
            dma((6,)), dma((_NS,)), dma((_NS,)), dma((_NS,)), dma((f // _WD_ROWS,)),
        ],
        compiler_params=pltpu.CompilerParams(
            vmem_limit_bytes=64 * 1024 * 1024,
            disable_semaphore_checks=True,
        ),
    )(A_x.reshape(1, d), kT, vT, A_wq, A_wo, B_w_gate, B_w_up, B_w_down, c, w_mod)
    return out.reshape(batch, sq, d)
```

```python
import functools

import jax
import jax.numpy as jnp
from jax import lax
from jax.experimental import pallas as pl
from jax.experimental.pallas import tpu as pltpu

_HQ, _DH = 32, 192
_G = 4
_NS = 2
_M = 8
_WD_ROWS = 128
_TAIL_ROWS = 128
_TAIL_STEP = 32
_EPS = 1e-5


def _dot(a, b):
    return jnp.dot(a, b, preferred_element_type=jnp.float32)


def _dot_nt(a, b):
    return lax.dot_general(a, b, (((1,), (1,)), ((), ())), preferred_element_type=jnp.float32)


def _layernorm(x):
    d = x - jnp.mean(x, axis=-1, keepdims=True)
    v = jnp.mean(d * d, axis=-1, keepdims=True)
    return d * lax.rsqrt(v + _EPS)


def _kernel(x_hbm, kT_hbm, vT_hbm, wq_hbm, wo_hbm, wg_hbm, wu_hbm, wd_hbm, c_hbm, wm_hbm,
            o_ref,
            x_v, c_v, wm_v, wq_v, wg_v, wu_v, wd_v, k_buf, v_buf, wo_buf, q_scr, hh_scr, hcol_scr,
            sem_w, sem_k, sem_v, sem_o, sem_d, sem_t, *, s0, w):
    f32, bf16 = jnp.float32, jnp.bfloat16
    n_groups = _HQ // _G
    gd = _G * _DH
    d = x_v.shape[-1]
    f = wd_v.shape[0]
    f_mxu = f - _TAIL_ROWS
    n_wd = f_mxu // _WD_ROWS
    n_tail = _TAIL_ROWS // _TAIL_STEP

    def group_rows(g):
        return pl.ds(pl.multiple_of(g * gd, 16), gd)

    def k_copy(g, slot):
        return pltpu.make_async_copy(kT_hbm.at[group_rows(g), pl.ds(s0, w)], k_buf.at[slot], sem_k.at[slot])

    def v_copy(g, slot):
        return pltpu.make_async_copy(vT_hbm.at[group_rows(g), pl.ds(s0, w)], v_buf.at[slot], sem_v.at[slot])

    def wo_copy(g, slot):
        return pltpu.make_async_copy(wo_hbm.at[group_rows(g), :], wo_buf.at[slot], sem_o.at[slot])

    def wd_copy(i):
        rows = pl.ds(pl.multiple_of(i * _WD_ROWS, _WD_ROWS), _WD_ROWS)
        return pltpu.make_async_copy(wd_hbm.at[rows, :], wd_v.at[rows, :], sem_d.at[i])

    def tail_copy(j):
        rows = pl.ds(pl.multiple_of(f_mxu + j * _TAIL_STEP, _TAIL_STEP), _TAIL_STEP)
        return pltpu.make_async_copy(wd_hbm.at[rows, :], wd_v.at[rows, :], sem_t.at[j])

    wm_copy = pltpu.make_async_copy(wm_hbm, wm_v, sem_w.at[0])
    c_copy = pltpu.make_async_copy(c_hbm, c_v, sem_w.at[1])
    x_copy = pltpu.make_async_copy(x_hbm, x_v, sem_w.at[2])
    wq_copy = pltpu.make_async_copy(wq_hbm, wq_v, sem_w.at[3])
    wg_copy = pltpu.make_async_copy(wg_hbm, wg_v, sem_w.at[4])
    wu_copy = pltpu.make_async_copy(wu_hbm, wu_v, sem_w.at[5])

    wm_copy.start()
    c_copy.start()
    x_copy.start()
    wq_copy.start()
    for g in range(_NS):
        k_copy(g, g).start()
        v_copy(g, g).start()
        wo_copy(g, g).start()

    c_copy.wait()
    wm_copy.wait()
    cc = jnp.broadcast_to(c_v[...].astype(f32), (_M, d))
    mod = _dot((cc * jax.nn.sigmoid(cc)).astype(bf16), wm_v[...])
    sa, ca, ga, sb, cb, gb = (mod[:, i * d:(i + 1) * d] for i in range(6))

    x_copy.wait()
    x = jnp.broadcast_to(x_v[...].astype(f32), (_M, d))
    h = (_layernorm(x) * (1.0 + ca) + sa).astype(bf16)

    row = lax.broadcasted_iota(jnp.int32, (_M, gd), 0)
    col = lax.broadcasted_iota(jnp.int32, (_M, gd), 1)
    block_diag = (col >= row * _DH) & (col < (row + 1) * _DH)
    wq_copy.wait()
    for g in range(n_groups):
        q = _dot(h, wq_v[:, g * gd:(g + 1) * gd])
        q_scr[g] = jnp.where(block_diag, q, 0.0).astype(bf16)

    def attend(g, acc):
        slot = g % _NS
        refill = g + _NS < n_groups

        k_copy(g, slot).wait()
        s = _dot(q_scr[g], k_buf[slot]) * (_DH ** -0.5)

        @pl.when(refill)
        def _():
            k_copy(g + _NS, slot).start()

        @pl.when(g + _NS == n_groups)
        def _():
            wg_copy.start()
            wu_copy.start()

            @pl.loop(0, n_wd)
            def _(i):
                wd_copy(i).start()

            @pl.loop(0, n_tail)
            def _(j):
                tail_copy(j).start()

        p = jnp.exp(s - jnp.max(s, axis=-1, keepdims=True))
        denom = jnp.sum(p, axis=-1, keepdims=True)

        v_copy(g, slot).wait()
        o = _dot_nt(p.astype(bf16), v_buf[slot])

        @pl.when(refill)
        def _():
            v_copy(g + _NS, slot).start()

        o = jnp.where(block_diag, o * (1.0 / denom), 0.0).astype(bf16)

        wo_copy(g, slot).wait()
        acc = acc + _dot(o, wo_buf[slot])

        @pl.when(refill)
        def _():
            wo_copy(g + _NS, slot).start()

        return acc

    acc = lax.fori_loop(0, n_groups, attend, jnp.zeros((_M, d), f32))
    attn = jnp.broadcast_to(jnp.sum(acc, axis=0, keepdims=True), (_M, d))
    x1 = x + ga * attn

    h2 = (_layernorm(x1) * (1.0 + cb) + sb).astype(bf16)
    wg_copy.wait()
    gate = _dot(h2, wg_v[...])
    wu_copy.wait()
    up = _dot(h2, wu_v[...])
    hh = (gate * up).astype(bf16)
    for i in range(n_wd):
        hh_scr[i] = hh[:, i * _WD_ROWS:(i + 1) * _WD_ROWS]

    hcol_scr[...] = jnp.broadcast_to(hh[:, f_mxu:].astype(f32).T[:, 0:1], (_TAIL_ROWS, 128))

    def down(i, y):
        wd_copy(i).wait()
        rows = pl.ds(pl.multiple_of(i * _WD_ROWS, _WD_ROWS), _WD_ROWS)
        return y + _dot(hh_scr[i], wd_v[rows, :])

    y = lax.fori_loop(0, n_wd, down, jnp.zeros((_M, d), f32))
    y = jnp.where(lax.broadcasted_iota(jnp.int32, (_M, d), 0) == 0, y, 0.0)
    for j in range(n_tail):
        r0 = j * _TAIL_STEP
        tail_copy(j).wait()
        hcol = hcol_scr[r0:r0 + _TAIL_STEP, :]
        blk = wd_v[f_mxu + r0:f_mxu + r0 + _TAIL_STEP, :].astype(f32)
        y = y + jnp.concatenate(
            [jnp.sum((blk[:, t:t + 128] * hcol).reshape(_TAIL_STEP // _M, _M, 128), axis=0)
             for t in range(0, d, 128)], axis=1)
    y = jnp.sum(y, axis=0, keepdims=True)
    o_ref[...] = (x1[0:1, :] + gb[0:1, :] * y).astype(o_ref.dtype)


@jax.jit
def pallas_adaLN_cond__sliding_block_cached__glu_gated_bilinear__decode_kernel(
    A_x: jax.Array,
    A_k_cache: jax.Array,
    A_v_cache: jax.Array,
    A_wq: jax.Array,
    A_wo: jax.Array,
    B_x: jax.Array,
    B_w_gate: jax.Array,
    B_w_up: jax.Array,
    B_w_down: jax.Array,
    c: jax.Array,
    w_mod: jax.Array,
):
    del B_x
    batch, sq, d = A_x.shape
    _, hkv, sk, dh = A_k_cache.shape
    f = B_w_gate.shape[1]
    w = min(4096, max(256, sk // 4))
    gd = _G * _DH
    assert (batch, sq) == (1, 1) and (hkv, dh) == (_HQ, _DH)
    assert gd % 128 == 0 and _G <= _M and _HQ % _G == 0 and d % 128 == 0
    assert (f - _TAIL_ROWS) % _WD_ROWS == 0 and _TAIL_ROWS == 128 and _TAIL_ROWS % _TAIL_STEP == 0
    assert w % 128 == 0 and (sk - w) % 128 == 0

    kT = jnp.swapaxes(A_k_cache.reshape(hkv, sk, dh), 1, 2).reshape(hkv * dh, sk)
    vT = jnp.swapaxes(A_v_cache.reshape(hkv, sk, dh), 1, 2).reshape(hkv * dh, sk)

    bf16 = jnp.bfloat16
    dma = pltpu.SemaphoreType.DMA
    out = pl.pallas_call(
        functools.partial(_kernel, s0=sk - w, w=w),
        out_shape=jax.ShapeDtypeStruct((1, d), A_x.dtype),
        in_specs=[pl.BlockSpec(memory_space=pl.ANY)] * 10,
        out_specs=pl.BlockSpec(memory_space=pltpu.VMEM),
        scratch_shapes=[
            pltpu.VMEM((1, d), bf16),
            pltpu.VMEM((1, d), bf16),
            pltpu.VMEM((d, 6 * d), bf16),
            pltpu.VMEM((d, _HQ * _DH), bf16),
            pltpu.VMEM((d, f), bf16),
            pltpu.VMEM((d, f), bf16),
            pltpu.VMEM((f, d), bf16),
            pltpu.VMEM((_NS, gd, w), bf16),
            pltpu.VMEM((_NS, gd, w), bf16),
            pltpu.VMEM((_NS, gd, d), bf16),
            pltpu.VMEM((_HQ // _G, _M, gd), bf16),
            pltpu.VMEM(((f - _TAIL_ROWS) // _WD_ROWS, _M, _WD_ROWS), bf16),
            pltpu.VMEM((_TAIL_ROWS, 128), jnp.float32),
            dma((6,)), dma((_NS,)), dma((_NS,)), dma((_NS,)),
            dma(((f - _TAIL_ROWS) // _WD_ROWS,)), dma((_TAIL_ROWS // _TAIL_STEP,)),
        ],
        compiler_params=pltpu.CompilerParams(
            vmem_limit_bytes=64 * 1024 * 1024,
            disable_semaphore_checks=True,
        ),
    )(A_x.reshape(1, d), kT, vT, A_wq, A_wo, B_w_gate, B_w_up, B_w_down, c, w_mod)
    return out.reshape(batch, sq, d)
```
